```python
import os as _os
_os.environ.setdefault('JAX_PLATFORMS', 'cpu')
import jax
import jax.numpy as jnp

def _softmax(x, axis=-1):
    return jax.nn.softmax(x, axis=axis)

def _gelu(x):
    return jax.nn.gelu(x, approximate=True)

def _silu(x):
    return jax.nn.silu(x)

def _sigmoid(x):
    return jax.nn.sigmoid(x)

def _layernorm(x, axis=-1, eps=1e-05):
    m = jnp.mean(x, axis=axis, keepdims=True)
    v = jnp.var(x, axis=axis, keepdims=True)
    return (x - m) / jnp.sqrt(v + eps)

def _scatter_add(tgt, idx, src, axis=0):
    return tgt.at[idx].add(src)

def _segment_sum(src, seg, n):
    return jax.ops.segment_sum(src, seg, n)

class _Rng:

    def __init__(self, key):
        self._k = key

    def _next(self):
        self._k, sub = jax.random.split(self._k)
        return sub

    def normal(self, shape):
        return jax.random.normal(self._next(), shape, dtype=jnp.bfloat16)

    def randint(self, lo, hi, shape):
        return jax.random.randint(self._next(), shape, lo, hi, dtype=jnp.int32)

    def uniform(self, shape, lo=0.0, hi=1.0):
        return jax.random.uniform(self._next(), shape, jnp.bfloat16, lo, hi)

    def permutation(self, n):
        return jax.random.permutation(self._next(), n)
kernel_name = 'adaLN_cond__mha_block_cached__geglu_ffn__prompt'

def setup_inputs():
    _rng = _Rng(jax.random.key(int.from_bytes(__import__("os").urandom(4), "little")))
    _w = lambda a: (lambda t: t.astype(jnp.bfloat16) if jnp.issubdtype(t.dtype, jnp.floating) else t)(jnp.asarray(a))

    def _A_setup():
        B, Sq, D = (1, 2048, 512)
        H, Sk, Dh = (32, 2048, 128)
        return {'x': _w((lambda *s: _rng.normal(s) * 0.05)(B, Sq, D)), 'k_cache': _w((lambda *s: _rng.normal(s) * 3.2)(B, H, Sk, Dh)), 'v_cache': _w((lambda *s: _rng.normal(s) * 0.4)(B, H, Sk, Dh)), 'wq': _w((lambda *s: _rng.normal(s) * 1.6)(D, H * Dh) * D ** (-0.5)), 'wo': _w((lambda *s: _rng.normal(s) * 0.4)(H * Dh, D) * (H * Dh) ** (-0.5))}
    _A_in = _A_setup()

    def _B_setup():
        B, S, D, F = (1, 2048, 512, 1792)
        return {'x': _w((lambda *s: _rng.normal(s) * 0.05)(B, S, D)), 'w_gate': _w((lambda *s: _rng.normal(s) * 0.05)(D, F)), 'w_up': _w((lambda *s: _rng.normal(s) * 0.05)(D, F)), 'w_down': _w((lambda *s: _rng.normal(s) * 0.05)(F, D))}
    _B_in = _B_setup()
    return {'A_x': _A_in['x'], 'A_k_cache': _A_in['k_cache'], 'A_v_cache': _A_in['v_cache'], 'A_wq': _A_in['wq'], 'A_wo': _A_in['wo'], 'B_x': _B_in['x'], 'B_w_gate': _B_in['w_gate'], 'B_w_up': _B_in['w_up'], 'B_w_down': _B_in['w_down'], 'c': _w((lambda *s: _rng.normal(s) * 0.05)(1, 512) * 8.0), 'w_mod': _w((lambda *s: _rng.normal(s) * 0.05)(512, 6 * 512) * 512 ** (-0.5) * 8.0)}

def reference(A_x, A_k_cache, A_v_cache, A_wq, A_wo, B_x, B_w_gate, B_w_up, B_w_down, c, w_mod):

    def _A_ref(x, k_cache, v_cache, wq, wo):
        B, Sq, D = x.shape
        H, Dh = (32, 128)
        q = (lambda x, *d: x.transpose(*d))((x @ wq).reshape(B, Sq, H, Dh), 0, 2, 1, 3)
        scores = jnp.einsum('bhqd,bhkd->bhqk', q, k_cache) * Dh ** (-0.5)
        p = _softmax(scores, axis=-1)
        o = jnp.einsum('bhqk,bhkd->bhqd', p, v_cache)
        return (lambda x, *d: x.transpose(*d))(o, 0, 2, 1, 3).reshape(B, Sq, H * Dh) @ wo

    def _B_ref(x, w_gate, w_up, w_down):
        return _gelu(x @ w_gate) * (x @ w_up) @ w_down
    x = A_x
    mod = (_silu(c) @ w_mod).reshape(c.shape[0], 6, 1, -1)
    sa, ca, ga, sb, cb, gb = (mod[:, 0].copy(), mod[:, 1].copy(), mod[:, 2].copy(), mod[:, 3].copy(), mod[:, 4].copy(), mod[:, 5].copy())
    h = _layernorm(x, axis=-1) * (1 + ca) + sa
    x = x + ga * _A_ref(h, A_k_cache, A_v_cache, A_wq, A_wo)
    h = _layernorm(x, axis=-1) * (1 + cb) + sb
    x = x + gb * _B_ref(h, B_w_gate, B_w_up, B_w_down)
    return x
```

```python
import functools

import jax
import jax.numpy as jnp
from jax import lax
import jax.experimental.pallas as pl
import jax.experimental.pallas.tpu as pltpu

_EPS = 1e-5
_F32 = jnp.float32
_BF16 = jnp.bfloat16


def _layernorm_rows(x):
    mu = jnp.mean(x, axis=-1, keepdims=True)
    xc = x - mu
    var = jnp.mean(xc * xc, axis=-1, keepdims=True)
    return xc * lax.rsqrt(var + _EPS)


def _kernel(x_ref, k_ref, v_ref, wq_ref, wo_ref, c_ref, wmod_ref, wg_ref, wu_ref, wd_ref,
            o_ref, mod_ref, h_ref, acc_ref, *, tq, n_heads, d_model, scale):
    hd = pl.program_id(0)
    i = pl.program_id(1)
    D = d_model
    rows = pl.ds(pl.multiple_of(i * tq, tq), tq)

    @pl.when(hd == 0)
    def _prologue():
        @pl.when(i == 0)
        def _mod():
            c = c_ref[...].astype(_F32)
            sc = c * jax.nn.sigmoid(c)
            sc8 = jnp.broadcast_to(sc, (8, D)).astype(_BF16)
            mod_ref[...] = jnp.dot(sc8, wmod_ref[...], preferred_element_type=_F32)

        x = x_ref[rows, :].astype(_F32)
        hn = _layernorm_rows(x)
        sa = mod_ref[0:1, 0:D]
        ca = mod_ref[0:1, D:2 * D]
        h_ref[rows, :] = (hn * (1.0 + ca) + sa).astype(_BF16)
        acc_ref[rows, :] = jnp.zeros((tq, D), _F32)

    h = h_ref[rows, :]
    q = jnp.dot(h, wq_ref[...], preferred_element_type=_F32)
    q = (q * scale).astype(_BF16)
    s = lax.dot_general(q, k_ref[0], (((1,), (1,)), ((), ())), preferred_element_type=_F32)
    m = jnp.max(s, axis=-1, keepdims=True)
    p = jnp.exp(s - m)
    l = jnp.sum(p, axis=-1, keepdims=True)
    o = jnp.dot(p.astype(_BF16), v_ref[0], preferred_element_type=_F32)
    o = o / l
    acc_ref[rows, :] += jnp.dot(o.astype(_BF16), wo_ref[...], preferred_element_type=_F32)

    @pl.when(hd == n_heads - 1)
    def _epilogue():
        x = x_ref[rows, :].astype(_F32)
        ga = mod_ref[0:1, 2 * D:3 * D]
        sb = mod_ref[0:1, 3 * D:4 * D]
        cb = mod_ref[0:1, 4 * D:5 * D]
        gb = mod_ref[0:1, 5 * D:6 * D]
        x1 = x + ga * acc_ref[rows, :]
        h2 = (_layernorm_rows(x1) * (1.0 + cb) + sb).astype(_BF16)
        g = jnp.dot(h2, wg_ref[...], preferred_element_type=_F32)
        u = jnp.dot(h2, wu_ref[...], preferred_element_type=_F32)
        a = (jax.nn.gelu(g, approximate=True) * u).astype(_BF16)
        ffn = jnp.dot(a, wd_ref[...], preferred_element_type=_F32)
        o_ref[...] = (x1 + gb * ffn).astype(o_ref.dtype)


@jax.jit
def pallas_adaLN_cond__mha_block_cached__geglu_ffn__prompt_kernel(
    A_x: jax.Array,
    A_k_cache: jax.Array,
    A_v_cache: jax.Array,
    A_wq: jax.Array,
    A_wo: jax.Array,
    B_x: jax.Array,
    B_w_gate: jax.Array,
    B_w_up: jax.Array,
    B_w_down: jax.Array,
    c: jax.Array,
    w_mod: jax.Array,
):
    del B_x
    B, S, D = A_x.shape
    _, H, SK, DH = A_k_cache.shape
    F = B_w_gate.shape[1]
    assert B == 1
    tq = 512
    nq = S // tq

    x2 = A_x.reshape(S, D)
    k3 = A_k_cache.reshape(H, SK, DH)
    v3 = A_v_cache.reshape(H, SK, DH)

    kern = functools.partial(_kernel, tq=tq, n_heads=H, d_model=D, scale=float(DH) ** -0.5)

    const2 = lambda h, i: (0, 0)
    out = pl.pallas_call(
        kern,
        grid=(H, nq),
        in_specs=[
            pl.BlockSpec((S, D), const2),
            pl.BlockSpec((1, SK, DH), lambda h, i: (h, 0, 0)),
            pl.BlockSpec((1, SK, DH), lambda h, i: (h, 0, 0)),
            pl.BlockSpec((D, DH), lambda h, i: (0, h)),
            pl.BlockSpec((DH, D), lambda h, i: (h, 0)),
            pl.BlockSpec((1, D), const2),
            pl.BlockSpec((D, 6 * D), const2),
            pl.BlockSpec((D, F), const2),
            pl.BlockSpec((D, F), const2),
            pl.BlockSpec((F, D), const2),
        ],
        out_specs=pl.BlockSpec((tq, D), lambda h, i: (jnp.where(h == H - 1, i, 0), 0)),
        out_shape=jax.ShapeDtypeStruct((S, D), A_x.dtype),
        scratch_shapes=[
            pltpu.VMEM((8, 6 * D), _F32),
            pltpu.VMEM((S, D), _BF16),
            pltpu.VMEM((S, D), _F32),
        ],
        compiler_params=pltpu.CompilerParams(
            dimension_semantics=("arbitrary", "arbitrary"),
            vmem_limit_bytes=100 * 1024 * 1024,
        ),
    )(x2, k3, v3, A_wq, A_wo, c, w_mod, B_w_gate, B_w_up, B_w_down)
    return out.reshape(B, S, D)
```

```python
import functools
import math
import jax
import jax.numpy as jnp
from jax import lax
import jax.experimental.pallas as pl
import jax.experimental.pallas.tpu as pltpu

_EPS = 1e-5
_F32 = jnp.float32
_BF16 = jnp.bfloat16


def _layernorm_rows(x):
    mu = jnp.mean(x, axis=-1, keepdims=True)
    xc = x - mu
    var = jnp.mean(xc * xc, axis=-1, keepdims=True)
    return xc * lax.rsqrt(var + _EPS)


def _kernel(x_ref, k_ref, v_ref, wq_ref, wo_ref, c_ref, wmod_ref, wg_hbm, wu_hbm, wd_hbm,
            o_ref, mod_ref, h_ref, acc_ref, wg_ref, wu_ref, wd_ref, sems, *, tq, ts, n_heads, d_model, scale):
    hd = pl.program_id(0)
    i = pl.program_id(1)
    D = d_model
    row0 = pl.multiple_of(i * tq, tq)
    rows = pl.ds(row0, tq)

    @pl.when(hd == 0)
    def _prologue():
        @pl.when(i == 0)
        def _mod():
            for n_, (src_, dst_) in enumerate(((wg_hbm, wg_ref), (wu_hbm, wu_ref), (wd_hbm, wd_ref))):
                pltpu.make_async_copy(src_, dst_, sems.at[n_]).start()
            c = c_ref[...].astype(_F32)
            sc = c * jax.nn.sigmoid(c)
            sc8 = jnp.broadcast_to(sc, (8, D)).astype(_BF16)
            mod_ref[...] = jnp.dot(sc8, wmod_ref[...], preferred_element_type=_F32)

        x = x_ref[rows, :].astype(_F32)
        hn = _layernorm_rows(x)
        sa = mod_ref[0:1, 0:D]
        ca = mod_ref[0:1, D:2 * D]
        h_ref[rows, :] = (hn * (1.0 + ca) + sa).astype(_BF16)
        acc_ref[rows, :] = jnp.zeros((tq, D), _F32)

    for j in range(tq // ts):
        r = pl.ds(pl.multiple_of(row0 + j * ts, ts), ts)
        h = h_ref[r, :]
        q = jnp.dot(h, wq_ref[...], preferred_element_type=_F32)
        q = (q * scale).astype(_BF16)
        s = lax.dot_general(q, k_ref[0], (((1,), (1,)), ((), ())), preferred_element_type=_F32)
        m = jnp.max(s, axis=-1, keepdims=True)
        p = jnp.exp2(s - m)
        l = jnp.sum(p, axis=-1, keepdims=True)
        o = jnp.dot(p.astype(_BF16), v_ref[0], preferred_element_type=_F32)
        o = o / l
        acc_ref[r, :] += jnp.dot(o.astype(_BF16), wo_ref[...], preferred_element_type=_F32)

    @pl.when(hd == n_heads - 1)
    def _epilogue():
        @pl.when(i == 0)
        def _wait_ffn_weights():
            for n_, (src_, dst_) in enumerate(((wg_hbm, wg_ref), (wu_hbm, wu_ref), (wd_hbm, wd_ref))):
                pltpu.make_async_copy(src_, dst_, sems.at[n_]).wait()

        x = x_ref[rows, :].astype(_F32)
        ga = mod_ref[0:1, 2 * D:3 * D]
        sb = mod_ref[0:1, 3 * D:4 * D]
        cb = mod_ref[0:1, 4 * D:5 * D]
        gb = mod_ref[0:1, 5 * D:6 * D]
        x1 = x + ga * acc_ref[rows, :]
        h2 = (_layernorm_rows(x1) * (1.0 + cb) + sb).astype(_BF16)
        g = jnp.dot(h2, wg_ref[...], preferred_element_type=_F32)
        u = jnp.dot(h2, wu_ref[...], preferred_element_type=_F32)
        a = (jax.nn.gelu(g, approximate=True) * u).astype(_BF16)
        ffn = jnp.dot(a, wd_ref[...], preferred_element_type=_F32)
        o_ref[...] = (x1 + gb * ffn).astype(o_ref.dtype)


@jax.jit
def pallas_adaLN_cond__mha_block_cached__geglu_ffn__prompt_kernel(
    A_x, A_k_cache, A_v_cache, A_wq, A_wo, B_x, B_w_gate, B_w_up, B_w_down, c, w_mod):
    del B_x
    B, S, D = A_x.shape
    _, H, SK, DH = A_k_cache.shape
    F = B_w_gate.shape[1]
    tq = 1024
    ts = 256
    nq = S // tq
    x2 = A_x.reshape(S, D)
    k3 = A_k_cache.reshape(H, SK, DH)
    v3 = A_v_cache.reshape(H, SK, DH)
    kern = functools.partial(_kernel, tq=tq, ts=ts, n_heads=H, d_model=D, scale=float(DH) ** -0.5 * math.log2(math.e))
    const2 = lambda h, i: (0, 0)
    out = pl.pallas_call(
        kern,
        grid=(H, nq),
        in_specs=[
            pl.BlockSpec((S, D), const2),
            pl.BlockSpec((1, SK, DH), lambda h, i: (h, 0, 0)),
            pl.BlockSpec((1, SK, DH), lambda h, i: (h, 0, 0)),
            pl.BlockSpec((D, DH), lambda h, i: (0, h)),
            pl.BlockSpec((DH, D), lambda h, i: (h, 0)),
            pl.BlockSpec((1, D), const2),
            pl.BlockSpec((D, 6 * D), const2),
            pl.BlockSpec(memory_space=pl.ANY),
            pl.BlockSpec(memory_space=pl.ANY),
            pl.BlockSpec(memory_space=pl.ANY),
        ],
        out_specs=pl.BlockSpec((tq, D), lambda h, i: (jnp.where(h == H - 1, i, 0), 0)),
        out_shape=jax.ShapeDtypeStruct((S, D), A_x.dtype),
        scratch_shapes=[
            pltpu.VMEM((8, 6 * D), _F32),
            pltpu.VMEM((S, D), _BF16),
            pltpu.VMEM((S, D), _F32),
            pltpu.VMEM((D, F), _BF16), pltpu.VMEM((D, F), _BF16), pltpu.VMEM((F, D), _BF16),
            pltpu.SemaphoreType.DMA((3,)),
        ],
        compiler_params=pltpu.CompilerParams(
            dimension_semantics=("arbitrary", "arbitrary"),
            vmem_limit_bytes=100 * 1024 * 1024,
        ),
    )(x2, k3, v3, A_wq, A_wo, c, w_mod, B_w_gate, B_w_up, B_w_down)
    return out.reshape(B, S, D)
```

```python
import functools
import math
import jax
import jax.numpy as jnp
from jax import lax
import jax.experimental.pallas as pl
import jax.experimental.pallas.tpu as pltpu

_EPS = 1e-5
_F32 = jnp.float32
_BF16 = jnp.bfloat16


def _layernorm_rows(x):
    mu = jnp.mean(x, axis=-1, keepdims=True)
    xc = x - mu
    var = jnp.mean(xc * xc, axis=-1, keepdims=True)
    return xc * lax.rsqrt(var + _EPS)


def _kernel(x_ref, k_ref, v_ref, wq_ref, wo_ref, c_ref, wmod_a_ref,
            wmod_hbm, wg_hbm, wu_hbm, wd_hbm, o_ref,
            mod_ref, h_ref, acc_ref, wmod_b_ref, wg_ref, wu_ref, wd_ref, sems,
            *, tq, tk, tf, n_heads, seq, d_model, scale):
    hd = pl.program_id(0)
    D = d_model

    def late_copies():
        return (
            pltpu.make_async_copy(wmod_hbm.at[:, pl.ds(2 * D, 4 * D)], wmod_b_ref, sems.at[0]),
            pltpu.make_async_copy(wg_hbm, wg_ref, sems.at[1]),
            pltpu.make_async_copy(wu_hbm, wu_ref, sems.at[2]),
            pltpu.make_async_copy(wd_hbm, wd_ref, sems.at[3]),
        )

    def silu_c():
        c = c_ref[...].astype(_F32)
        sc = c * jax.nn.sigmoid(c)
        return jnp.broadcast_to(sc, (8, D)).astype(_BF16)

    @pl.when(hd == 0)
    def _prologue():
        for cp in late_copies():
            cp.start()
        mod_ref[:, 0:2 * D] = jnp.dot(silu_c(), wmod_a_ref[...], preferred_element_type=_F32)
        sa = mod_ref[0:1, 0:D]
        ca = mod_ref[0:1, D:2 * D]

        def ln_body(b, carry):
            r = pl.ds(pl.multiple_of(b * tf, tf), tf)
            hn = _layernorm_rows(x_ref[r, :].astype(_F32))
            h_ref[r, :] = (hn * (1.0 + ca) + sa).astype(_BF16)
            acc_ref[r, :] = jnp.zeros((tf, D), _F32)
            return carry

        lax.fori_loop(0, seq // tf, ln_body, 0)

    def attn_body(i, carry):
        r = pl.ds(pl.multiple_of(i * tq, tq), tq)
        q = jnp.dot(h_ref[r, :], wq_ref[...], preferred_element_type=_F32)
        q = (q * scale).astype(_BF16)
        m = l = o = None
        for cc in range(0, k_ref.shape[1], tk):
            s = lax.dot_general(q, k_ref[0, cc:cc + tk, :], (((1,), (1,)), ((), ())),
                                preferred_element_type=_F32)
            m_cur = jnp.max(s, axis=-1, keepdims=True)
            if m is None:
                m = m_cur
                p = jnp.exp2(s - m)
                l = jnp.sum(p, axis=-1, keepdims=True)
                o = jnp.dot(p.astype(_BF16), v_ref[0, cc:cc + tk, :], preferred_element_type=_F32)
            else:
                m_new = jnp.maximum(m, m_cur)
                alpha = jnp.exp2(m - m_new)
                p = jnp.exp2(s - m_new)
                l = alpha * l + jnp.sum(p, axis=-1, keepdims=True)
                o = alpha * o + jnp.dot(p.astype(_BF16), v_ref[0, cc:cc + tk, :],
                                        preferred_element_type=_F32)
                m = m_new
        o = o / l
        acc_ref[r, :] += jnp.dot(o.astype(_BF16), wo_ref[...], preferred_element_type=_F32)
        return carry

    lax.fori_loop(0, seq // tq, attn_body, 0)

    @pl.when(hd == n_heads - 1)
    def _epilogue():
        for cp in late_copies():
            cp.wait()
        mod_ref[:, 2 * D:6 * D] = jnp.dot(silu_c(), wmod_b_ref[...], preferred_element_type=_F32)
        ga = mod_ref[0:1, 2 * D:3 * D]
        sb = mod_ref[0:1, 3 * D:4 * D]
        cb = mod_ref[0:1, 4 * D:5 * D]
        gb = mod_ref[0:1, 5 * D:6 * D]

        def ffn_body(b, carry):
            r = pl.ds(pl.multiple_of(b * tf, tf), tf)
            x1 = x_ref[r, :].astype(_F32) + ga * acc_ref[r, :]
            h2 = (_layernorm_rows(x1) * (1.0 + cb) + sb).astype(_BF16)
            g = jnp.dot(h2, wg_ref[...], preferred_element_type=_F32)
            u = jnp.dot(h2, wu_ref[...], preferred_element_type=_F32)
            a = (jax.nn.gelu(g, approximate=True) * u).astype(_BF16)
            ffn = jnp.dot(a, wd_ref[...], preferred_element_type=_F32)
            o_ref[r, :] = (x1 + gb * ffn).astype(o_ref.dtype)
            return carry

        lax.fori_loop(0, seq // tf, ffn_body, 0)


@jax.jit
def pallas_adaLN_cond__mha_block_cached__geglu_ffn__prompt_kernel(
    A_x, A_k_cache, A_v_cache, A_wq, A_wo, B_x, B_w_gate, B_w_up, B_w_down, c, w_mod):
    del B_x
    B, S, D = A_x.shape
    _, H, SK, DH = A_k_cache.shape
    F = B_w_gate.shape[1]
    tq = 1024
    tk = 512
    tf = 512
    x2 = A_x.reshape(S, D)
    k3 = A_k_cache.reshape(H, SK, DH)
    v3 = A_v_cache.reshape(H, SK, DH)
    kern = functools.partial(_kernel, tq=tq, tk=tk, tf=tf, n_heads=H, seq=S, d_model=D,
                             scale=float(DH) ** -0.5 * math.log2(math.e))
    const2 = lambda h: (0, 0)
    out = pl.pallas_call(
        kern,
        grid=(H,),
        in_specs=[
            pl.BlockSpec((S, D), const2),
            pl.BlockSpec((1, SK, DH), lambda h: (h, 0, 0)),
            pl.BlockSpec((1, SK, DH), lambda h: (h, 0, 0)),
            pl.BlockSpec((D, DH), lambda h: (0, h)),
            pl.BlockSpec((DH, D), lambda h: (h, 0)),
            pl.BlockSpec((1, D), const2),
            pl.BlockSpec((D, 2 * D), const2),
            pl.BlockSpec(memory_space=pl.ANY),
            pl.BlockSpec(memory_space=pl.ANY),
            pl.BlockSpec(memory_space=pl.ANY),
            pl.BlockSpec(memory_space=pl.ANY),
        ],
        out_specs=pl.BlockSpec((S, D), const2),
        out_shape=jax.ShapeDtypeStruct((S, D), A_x.dtype),
        scratch_shapes=[
            pltpu.VMEM((8, 6 * D), _F32),
            pltpu.VMEM((S, D), _BF16),
            pltpu.VMEM((S, D), _F32),
            pltpu.VMEM((D, 4 * D), _BF16),
            pltpu.VMEM((D, F), _BF16), pltpu.VMEM((D, F), _BF16), pltpu.VMEM((F, D), _BF16),
            pltpu.SemaphoreType.DMA((4,)),
        ],
        compiler_params=pltpu.CompilerParams(
            dimension_semantics=("arbitrary",),
            vmem_limit_bytes=100 * 1024 * 1024,
        ),
    )(x2, k3, v3, A_wq, A_wo, c, w_mod, w_mod, B_w_gate, B_w_up, B_w_down)
    return out.reshape(B, S, D)
```
